```python
import os as _os
_os.environ.setdefault("JAX_PLATFORMS", "cpu")
import jax
import jax.numpy as jnp

def _softmax(x, axis=-1):
    return jax.nn.softmax(x, axis=axis)
def _gelu(x):
    return jax.nn.gelu(x, approximate=True)
def _silu(x):
    return jax.nn.silu(x)
def _sigmoid(x):
    return jax.nn.sigmoid(x)
def _layernorm(x, axis=-1, eps=1e-5):
    m = jnp.mean(x, axis=axis, keepdims=True)
    v = jnp.var(x, axis=axis, keepdims=True)
    return (x - m) / jnp.sqrt(v + eps)
def _scatter_add(tgt, idx, src, axis=0):
    return tgt.at[idx].add(src)
def _segment_sum(src, seg, n):
    return jax.ops.segment_sum(src, seg, n)
class _Rng:
    def __init__(self, key):
        self._k = key
    def _next(self):
        self._k, sub = jax.random.split(self._k)
        return sub
    def normal(self, shape):
        return jax.random.normal(self._next(), shape, dtype=jnp.bfloat16)
    def randint(self, lo, hi, shape):
        return jax.random.randint(self._next(), shape, lo, hi, dtype=jnp.int32)
    def uniform(self, shape, lo=0.0, hi=1.0):
        return jax.random.uniform(self._next(), shape, jnp.bfloat16, lo, hi)
    def permutation(self, n):
        return jax.random.permutation(self._next(), n)


kernel_name = 'standalone__gqa_block_cached__sampling'

def setup_inputs():
    _rng = _Rng(jax.random.key(int.from_bytes(__import__("os").urandom(4), "little")))
    _w = (lambda a: (lambda t: t.astype(jnp.bfloat16) if jnp.issubdtype(t.dtype, jnp.floating) else t)(jnp.asarray(a)))
    B, Sq, D = 32, 16, 1024
    Hq, Hkv, Sk, Dh = 32, 4, 2048, 128
    assert Hq % Hkv == 0, (Hq, Hkv)
    return {
        "x": _w((lambda *s: _rng.normal(s) * 0.8)(B, Sq, D)),
        "k_cache": _w((lambda *s: _rng.normal(s) * 0.8)(B, Hkv, Sk, Dh)),
        "v_cache": _w((lambda *s: _rng.normal(s) * 0.05)(B, Hkv, Sk, Dh)),
        "wq": _w((lambda *s: _rng.normal(s) * 0.8)(D, Hq * Dh) * (D ** -0.5)),
        "wo": _w((lambda *s: _rng.normal(s) * 0.05)(Hq * Dh, D) * ((Hq * Dh) ** -0.5)),
    }

def reference(x, k_cache, v_cache, wq, wo):
    B, Sq, D = x.shape
    Hq, Dh = 32, 128
    Hkv = k_cache.shape[1]
    rep = Hq // Hkv
    q = (lambda x, *d: x.transpose(*d))((x @ wq).reshape(B, Sq, Hq, Dh), 0, 2, 1, 3)
    k = jnp.repeat(k_cache, rep, axis=1)
    v = jnp.repeat(v_cache, rep, axis=1)
    scores = jnp.einsum("bhqd,bhkd->bhqk", q, k) * (Dh ** -0.5)
    p = _softmax(scores, axis=-1)
    o = jnp.einsum("bhqk,bhkd->bhqd", p, v)
    return (lambda x, *d: x.transpose(*d))(o, 0, 2, 1, 3).reshape(B, Sq, Hq * Dh) @ wo
```

```python
import functools

import jax
import jax.numpy as jnp
from jax import lax
import jax.experimental.pallas as pl
import jax.experimental.pallas.tpu as pltpu

_RING = 6
_GB = 8


def _gqa_kernel(x_hbm, k_hbm, v_hbm, wq_hbm, wo_hbm, out_hbm,
                x_buf, wq_buf, wo_buf, kbuf, vbuf, q_buf, o_buf, acc, out_stage,
                kv_sems, w_sems, out_sems, *, B, SQ, HKV, REP, DH):
    G = REP * DH
    NG = B // _GB
    NCHUNK = NG * HKV
    NU = B * HKV
    R = _RING
    scale = DH ** -0.5

    def unit_bh(u):
        c = u // _GB
        j = u % _GB
        return (c // HKV) * _GB + j, c % HKV

    def k_copy(u):
        b, h = unit_bh(u)
        slot = u % R
        return pltpu.make_async_copy(k_hbm.at[b, h], kbuf.at[slot], kv_sems.at[0, slot])

    def v_copy(u):
        b, h = unit_bh(u)
        slot = u % R
        return pltpu.make_async_copy(v_hbm.at[b, h], vbuf.at[slot], kv_sems.at[1, slot])

    def x_copy():
        return pltpu.make_async_copy(x_hbm, x_buf, w_sems.at[0])

    def wq_copy(h):
        return pltpu.make_async_copy(wq_hbm.at[:, pl.ds(h * G, G)], wq_buf.at[h], w_sems.at[1 + h])

    def wo_copy(h):
        return pltpu.make_async_copy(wo_hbm.at[pl.ds(h * G, G), :], wo_buf.at[h],
                                     w_sems.at[1 + HKV + h])

    def out_copy(g):
        return pltpu.make_async_copy(out_stage.at[g],
                                     out_hbm.at[pl.ds(g * _GB * SQ, _GB * SQ), :],
                                     out_sems.at[g])

    x_copy().start()
    wq_copy(0).start()
    for u in range(R):
        k_copy(u).start()
        v_copy(u).start()
    for h in range(1, HKV):
        wq_copy(h).start()
    for h in range(HKV):
        wo_copy(h).start()

    def qk(c, j):
        slot = (c * _GB + j) % R
        qg = q_buf[j * SQ:(j + 1) * SQ, :]
        q = jnp.concatenate([qg[:, r * DH:(r + 1) * DH] for r in range(REP)], axis=0)
        return lax.dot_general(q, kbuf[slot], (((1,), (1,)), ((), ())),
                               preferred_element_type=jnp.float32)

    def softmax_pv(c, j, s):
        slot = (c * _GB + j) % R
        m = jnp.max(s, axis=1, keepdims=True)
        p = jnp.exp((s - m) * scale)
        l = jnp.sum(p, axis=1, keepdims=True)
        o = jnp.dot(p.astype(jnp.bfloat16), vbuf[slot], preferred_element_type=jnp.float32)
        o = (o / l).astype(o_buf.dtype)
        o_buf[j * SQ:(j + 1) * SQ, :] = jnp.concatenate(
            [o[r * SQ:(r + 1) * SQ, :] for r in range(REP)], axis=1)

    def chunk_body(c, carry):
        g = c // HKV
        h = c % HKV

        @pl.when(c == 0)
        def _():
            x_copy().wait()

        for hh in range(HKV):
            @pl.when(c == hh)
            def _():
                wq_copy(hh).wait()

        xg = x_buf[pl.ds(pl.multiple_of(g * _GB * SQ, _GB * SQ), _GB * SQ), :]
        q_buf[...] = jnp.dot(xg, wq_buf[h],
                             preferred_element_type=jnp.float32).astype(q_buf.dtype)

        k_copy(c * _GB).wait()
        s_cur = qk(c, 0)
        for j in range(_GB):
            u = c * _GB + j
            if j + 1 < _GB:
                k_copy(u + 1).wait()
            v_copy(u).wait()
            s_nxt = qk(c, j + 1) if j + 1 < _GB else None
            softmax_pv(c, j, s_cur)
            s_cur = s_nxt

            @pl.when(u + R < NU)
            def _():
                k_copy(u + R).start()
                v_copy(u + R).start()

        for hh in range(HKV):
            @pl.when(c == hh)
            def _():
                wo_copy(hh).wait()

        part = jnp.dot(o_buf[...], wo_buf[h], preferred_element_type=jnp.float32)

        @pl.when(h == 0)
        def _():
            acc[...] = part

        @pl.when(h > 0)
        def _():
            acc[...] += part

        @pl.when(h == HKV - 1)
        def _():
            out_stage[g] = acc[...].astype(out_stage.dtype)
            out_copy(g).start()

        return carry

    lax.fori_loop(0, NCHUNK, chunk_body, 0)
    for g in range(NG):
        out_copy(g).wait()


@jax.jit
def pallas_standalone__gqa_block_cached__sampling_kernel(
    x: jax.Array,
    k_cache: jax.Array,
    v_cache: jax.Array,
    wq: jax.Array,
    wo: jax.Array,
):
    B, SQ, D = x.shape
    _, HKV, SK, DH = k_cache.shape
    HQ = wq.shape[1] // DH
    REP = HQ // HKV
    G = REP * DH
    NG = B // _GB
    x2 = x.reshape(B * SQ, D)
    kernel = functools.partial(_gqa_kernel, B=B, SQ=SQ, HKV=HKV, REP=REP, DH=DH)
    out = pl.pallas_call(
        kernel,
        in_specs=[pl.BlockSpec(memory_space=pl.ANY)] * 5,
        out_specs=pl.BlockSpec(memory_space=pl.ANY),
        out_shape=jax.ShapeDtypeStruct((B * SQ, D), x.dtype),
        scratch_shapes=[
            pltpu.VMEM((B * SQ, D), x.dtype),
            pltpu.VMEM((HKV, D, G), wq.dtype),
            pltpu.VMEM((HKV, G, D), wo.dtype),
            pltpu.VMEM((_RING, SK, DH), k_cache.dtype),
            pltpu.VMEM((_RING, SK, DH), v_cache.dtype),
            pltpu.VMEM((_GB * SQ, G), jnp.bfloat16),
            pltpu.VMEM((_GB * SQ, G), jnp.bfloat16),
            pltpu.VMEM((_GB * SQ, D), jnp.float32),
            pltpu.VMEM((NG, _GB * SQ, D), x.dtype),
            pltpu.SemaphoreType.DMA((2, _RING)),
            pltpu.SemaphoreType.DMA((1 + 2 * HKV,)),
            pltpu.SemaphoreType.DMA((NG,)),
        ],
        compiler_params=pltpu.CompilerParams(vmem_limit_bytes=64 * 1024 * 1024),
    )(x2, k_cache, v_cache, wq, wo)
    return out.reshape(B, SQ, D)
```
